```python
import os as _os
_os.environ.setdefault("JAX_PLATFORMS", "cpu")
import jax
import jax.numpy as jnp

def _softmax(x, axis=-1):
    return jax.nn.softmax(x, axis=axis)
def _gelu(x):
    return jax.nn.gelu(x, approximate=True)
def _silu(x):
    return jax.nn.silu(x)
def _sigmoid(x):
    return jax.nn.sigmoid(x)
def _layernorm(x, axis=-1, eps=1e-5):
    m = jnp.mean(x, axis=axis, keepdims=True)
    v = jnp.var(x, axis=axis, keepdims=True)
    return (x - m) / jnp.sqrt(v + eps)
def _scatter_add(tgt, idx, src, axis=0):
    return tgt.at[idx].add(src)
def _segment_sum(src, seg, n):
    return jax.ops.segment_sum(src, seg, n)
class _Rng:
    def __init__(self, key):
        self._k = key
    def _next(self):
        self._k, sub = jax.random.split(self._k)
        return sub
    def normal(self, shape):
        return jax.random.normal(self._next(), shape, dtype=jnp.bfloat16)
    def randint(self, lo, hi, shape):
        return jax.random.randint(self._next(), shape, lo, hi, dtype=jnp.int32)
    def uniform(self, shape, lo=0.0, hi=1.0):
        return jax.random.uniform(self._next(), shape, jnp.bfloat16, lo, hi)
    def permutation(self, n):
        return jax.random.permutation(self._next(), n)


kernel_name = 'concat_heads__gqa_block_cached__gqa_block_cached__near_ridge'

def setup_inputs():
    _rng = _Rng(jax.random.key(int.from_bytes(__import__("os").urandom(4), "little")))
    _w = (lambda a: (lambda t: t.astype(jnp.bfloat16) if jnp.issubdtype(t.dtype, jnp.floating) else t)(jnp.asarray(a)))
    def _A_setup():
        B, Sq, D = 32, 48, 512
        Hq, Hkv, Sk, Dh = 32, 32, 48, 128
        assert Hq % Hkv == 0, (Hq, Hkv)
        return {
            "x": _w((lambda *s: _rng.normal(s) * 0.8)(B, Sq, D)),
            "k_cache": _w((lambda *s: _rng.normal(s) * 0.8)(B, Hkv, Sk, Dh)),
            "v_cache": _w((lambda *s: _rng.normal(s) * 0.05)(B, Hkv, Sk, Dh)),
            "wq": _w((lambda *s: _rng.normal(s) * 0.8)(D, Hq * Dh) * (D ** -0.5)),
            "wo": _w((lambda *s: _rng.normal(s) * 0.05)(Hq * Dh, D) * ((Hq * Dh) ** -0.5)),
        }
    _A_in = _A_setup()

    def _B_setup():
        B, Sq, D = 32, 48, 512
        Hq, Hkv, Sk, Dh = 32, 32, 48, 128
        assert Hq % Hkv == 0, (Hq, Hkv)
        return {
            "x": _w((lambda *s: _rng.normal(s) * 0.8)(B, Sq, D)),
            "k_cache": _w((lambda *s: _rng.normal(s) * 0.8)(B, Hkv, Sk, Dh)),
            "v_cache": _w((lambda *s: _rng.normal(s) * 0.05)(B, Hkv, Sk, Dh)),
            "wq": _w((lambda *s: _rng.normal(s) * 0.8)(D, Hq * Dh) * (D ** -0.5)),
            "wo": _w((lambda *s: _rng.normal(s) * 0.05)(Hq * Dh, D) * ((Hq * Dh) ** -0.5)),
        }
    _B_in = _B_setup()

    return {
        "A_x": _A_in["x"],
        "A_k_cache": _A_in["k_cache"],
        "A_v_cache": _A_in["v_cache"],
        "A_wq": _A_in["wq"],
        "A_wo": _A_in["wo"],
        "B_x": _B_in["x"],
        "B_k_cache": _B_in["k_cache"],
        "B_v_cache": _B_in["v_cache"],
        "B_wq": _B_in["wq"],
        "B_wo": _B_in["wo"],
    }

def reference(A_x, A_k_cache, A_v_cache, A_wq, A_wo, B_x, B_k_cache, B_v_cache, B_wq, B_wo):
    def _A_ref(x, k_cache, v_cache, wq, wo):
        B, Sq, D = x.shape
        Hq, Dh = 32, 128
        Hkv = k_cache.shape[1]
        rep = Hq // Hkv
        q = (lambda x, *d: x.transpose(*d))((x @ wq).reshape(B, Sq, Hq, Dh), 0, 2, 1, 3)
        k = jnp.repeat(k_cache, rep, axis=1)
        v = jnp.repeat(v_cache, rep, axis=1)
        scores = jnp.einsum("bhqd,bhkd->bhqk", q, k) * (Dh ** -0.5)
        p = _softmax(scores, axis=-1)
        o = jnp.einsum("bhqk,bhkd->bhqd", p, v)
        return (lambda x, *d: x.transpose(*d))(o, 0, 2, 1, 3).reshape(B, Sq, Hq * Dh) @ wo

    def _B_ref(x, k_cache, v_cache, wq, wo):
        B, Sq, D = x.shape
        Hq, Dh = 32, 128
        Hkv = k_cache.shape[1]
        rep = Hq // Hkv
        q = (lambda x, *d: x.transpose(*d))((x @ wq).reshape(B, Sq, Hq, Dh), 0, 2, 1, 3)
        k = jnp.repeat(k_cache, rep, axis=1)
        v = jnp.repeat(v_cache, rep, axis=1)
        scores = jnp.einsum("bhqd,bhkd->bhqk", q, k) * (Dh ** -0.5)
        p = _softmax(scores, axis=-1)
        o = jnp.einsum("bhqk,bhkd->bhqd", p, v)
        return (lambda x, *d: x.transpose(*d))(o, 0, 2, 1, 3).reshape(B, Sq, Hq * Dh) @ wo

    a = _A_ref(A_x, A_k_cache, A_v_cache, A_wq, A_wo)
    b = _B_ref(B_x, B_k_cache, B_v_cache, B_wq, B_wo)
    return jnp.concatenate([a, b], axis=-1)
```

```python
import functools, math, contextlib
import jax
import jax.numpy as jnp
from jax import lax
import jax.experimental.pallas as pl
import jax.experimental.pallas.tpu as pltpu

B, SQ, D = 32, 48, 512
H, SK, DH = 32, 48, 128
C2 = (DH ** -0.5) * math.log2(math.e)
BB = 4
HG = 4
NT = B // BB
NG = H // HG
W = HG * DH
M = BB * SQ
NTILES = 2 * NT * NG
BF = jnp.bfloat16
F32 = jnp.float32
P, L, E = 12, 8, 4
NB = (NTILES - P - E) // L
S_KV, S_W, S_HU5, S_B, S_OUT, NSEM = 6, 20, 26, 27, 28, 29


def tile_coords(i):
    if isinstance(i, int):
        br, hi, lo = i >> 6, (i >> 3) & 7, i & 7
        return (br, lo, hi) if br == 0 else (br, hi, lo)
    br = lax.shift_right_logical(i, 6)
    hi = lax.shift_right_logical(i, 3) & 7
    lo = i & 7
    t = jnp.where(br == 0, lo, hi)
    g = jnp.where(br == 0, hi, lo)
    return br, t, g


def kern(ax, ak, av, awq, awo, bx, bk, bv, bwq, bwo, out_hbm,
         x_buf, k_buf, v_buf, wq_buf, wo_buf, acc_ref, stage, q_car, o_car, sem, *, scopes, endq):
    scope = jax.named_scope if scopes else (lambda n: contextlib.nullcontext())
    cp = pltpu.make_async_copy
    def xa(t0, n, s):
        return cp(ax.at[pl.ds(t0 * BB, n * BB)], x_buf.at[0, pl.ds(t0 * BB, n * BB)], sem.at[s])
    def kva(g, t0, n, s):
        return [cp(src.at[pl.ds(t0 * BB, n * BB), pl.ds(g * HG, HG)],
                   buf.at[0, pl.ds(t0 * BB, n * BB), pl.ds(g * HG, HG)], sem.at[s]) for src, buf in ((ak, k_buf), (av, v_buf))]
    def hu_a(hu, s):
        return kva(hu // 2, (hu % 2) * 4, 4, s)
    def kvb(t, s):
        return [cp(src.at[pl.ds(t * BB, BB)], buf.at[1, pl.ds(t * BB, BB)], sem.at[s]) for src, buf in ((bk, k_buf), (bv, v_buf))]
    def wqc(br, g, s):
        return cp((awq, bwq)[br].at[:, pl.ds(g * W, W)], wq_buf.at[br, g], sem.at[s])
    def woa(g, s):
        return cp(awo.at[pl.ds(g * W, W), :], wo_buf.at[0, pl.ds(g * W, W)], sem.at[s])

    groups = [
        [wqc(0, 0, 0), xa(0, 1, 0)],
        [xa(1, 2, 1)],
        [xa(3, 5, 2)],
        hu_a(0, 3) + [woa(0, 3)],
        hu_a(1, 4) + [wqc(0, 1, 4)],
        hu_a(2, 5) + [woa(1, 5)],
    ]
    for grp in groups:
        for c in grp:
            c.start()
    for c in hu_a(3, S_KV) + [wqc(0, 2, S_W)] + hu_a(4, S_KV) + [woa(2, S_W)]:
        c.start()
    hu5 = hu_a(5, S_HU5)
    for c in hu5:
        c.start()
    for j in range(1, 6):
        for c in [wqc(0, j + 2, S_W + j), woa(j + 2, S_W + j)] + kva(j + 2, 0, NT, S_KV + j):
            c.start()
    bgrp = [cp(bx, x_buf.at[1], sem.at[S_B]), cp(bwo, wo_buf.at[1], sem.at[S_B])]
    for c in bgrp:
        c.start()
    for g in range(NG):
        wqc(1, g, S_B).start()
    for t in range(NT):
        for c in kvb(t, S_KV + 6 + t):
            c.start()

    def wait_group(n):
        with scope(f"W{n}"):
            for c in groups[n]:
                c.wait()

    q = {}; er = {}; o = {}

    def Q(i, key):
        br, t, g = tile_coords(i)
        x = x_buf[br, pl.ds(t * BB, BB)].reshape(M, D)
        qq = jnp.dot(x, wq_buf[br, g], preferred_element_type=F32)
        q[key] = {(b, hh): qq[b * SQ:(b + 1) * SQ, hh * DH:(hh + 1) * DH].astype(BF)
                  for hh in range(HG) for b in range(BB)}

    def S(i, key):
        br, t, g = tile_coords(i)
        d = {}
        for hh in range(HG):
            for b in range(BB):
                s = lax.dot_general(q[key][b, hh], k_buf[br, t * BB + b, g * HG + hh],
                                    (((1,), (1,)), ((), ())), preferred_element_type=F32)
                m = jnp.max(s, axis=-1, keepdims=True)
                e = jnp.exp2((s - m) * C2)
                l = jnp.sum(e, axis=-1, keepdims=True)
                d[b, hh] = (e.astype(BF), pl.reciprocal(l, approx=True))
        er[key] = d
        del q[key]

    def Pv(i, key):
        br, t, g = tile_coords(i)
        d = {}
        for hh in range(HG):
            for b in range(BB):
                e, r = er[key][b, hh]
                oo = jnp.dot(e, v_buf[br, t * BB + b, g * HG + hh], preferred_element_type=F32)
                d[b, hh] = (oo * r).astype(BF)
        rows = [jnp.concatenate([d[b, hh] for hh in range(HG)], axis=1) for b in range(BB)]
        o[key] = jnp.concatenate(rows, axis=0)
        del er[key]

    def O(i, key):
        br, t, g = tile_coords(i)
        if isinstance(i, int):
            p = jnp.dot(o[key], wo_buf[br, g * W:(g + 1) * W], preferred_element_type=F32)
            a = p if g == 0 else acc_ref[t] + p
            if g < NG - 1:
                acc_ref[t] = a
            else:
                stage[br, pl.ds(t * BB, BB)] = a.astype(BF).reshape(BB, SQ, D)
        else:
            p = jnp.dot(o[key], wo_buf[br, pl.ds(pl.multiple_of(g * W, W), W)], preferred_element_type=F32)
            a = jnp.where(g == 0, 0.0, acc_ref[t]) + p
            acc_ref[t] = a
            stage[br, pl.ds(t * BB, BB)] = a.astype(BF).reshape(BB, SQ, D)
        del o[key]

    def save_carry(k0):
        for j in range(2):
            for (b, hh), val in q[k0 + j].items():
                q_car[j, b, hh] = val
            del q[k0 + j]
        o_car[...] = o[k0 - 1]
        del o[k0 - 1]

    def load_carry(k0):
        for j in range(2):
            q[k0 + j] = {(b, hh): q_car[j, b, hh] for hh in range(HG) for b in range(BB)}
        o[k0 - 1] = o_car[...]

    def out_a():
        return cp(stage.at[0], out_hbm.at[:, :, pl.ds(0, D)], sem.at[S_OUT])
    def out_b(t):
        return cp(stage.at[1, pl.ds(t * BB, BB)], out_hbm.at[pl.ds(t * BB, BB), :, pl.ds(D, D)], sem.at[S_OUT])

    def iters(base, k0, n):
        for k in range(k0, k0 + n):
            i = base + k
            S(i, k); O(i - 1, k - 1)
            if endq and k == k0 + n - 1:
                Pv(i, k); Q(i + 2, k + 2)
            else:
                Q(i + 2, k + 2); Pv(i, k)

    wait_group(0)
    Q(0, 0)
    wait_group(1)
    Q(1, 1); Q(2, 2)
    wait_group(2)
    for i in range(3, 8):
        Q(i, i)
    wait_group(3)
    S(0, 0); S(1, 1); Pv(0, 0); S(2, 2); O(0, 0); Pv(1, 1); S(3, 3); O(1, 1); Pv(2, 2); Pv(3, 3); O(2, 2)
    wait_group(4)
    S(4, 4); O(3, 3); S(5, 5); Q(8, 8); Pv(4, 4); S(6, 6); O(4, 4); Pv(5, 5); S(7, 7); O(5, 5); Pv(6, 6); O(6, 6); Pv(7, 7); Q(9, 9)
    wait_group(5)
    iters(0, 8, 4)
    save_carry(12)

    def body(j, carry):
        base = P + j * L
        with scope("WL"):
            cp(ak.at[pl.ds(0, 2 * BB)], k_buf.at[0, pl.ds(0, 2 * BB)], sem.at[S_KV + j]).wait()
            @pl.when(j < 6)
            def _():
                cp(awo.at[pl.ds(0, 2 * W)], wo_buf.at[0, pl.ds(0, 2 * W)], sem.at[S_W + j]).wait()
            @pl.when(j == 1)
            def _():
                cp(ak.at[pl.ds(0, BB)], k_buf.at[0, pl.ds(0, BB)], sem.at[S_HU5]).wait()
            @pl.when(j == 6)
            def _():
                for c in bgrp:
                    c.wait()
                cp(bwo, wo_buf.at[1], sem.at[S_B]).wait()
        load_carry(0)
        iters(base, 0, L)
        save_carry(L)
        @pl.when(j == 6)
        def _():
            out_a().start()
        @pl.when(j >= 7)
        def _():
            out_b(j - 7).start()
        return carry
    lax.fori_loop(0, NB, body, 0)

    base = NTILES - E
    with scope("EP"):
        pass
    load_carry(base)
    for i in range(base, NTILES):
        S(i, i); O(i - 1, i - 1)
        if i + 2 < NTILES:
            Q(i + 2, i + 2)
        Pv(i, i)
    O(NTILES - 1, NTILES - 1)
    out_b(NT - 1).start()
    with scope("WO"):
        out_a().wait()
        for t in range(NT):
            out_b(t).wait()


@jax.jit
def pallas_concat_heads__gqa_block_cached__gqa_block_cached__near_ridge_kernel(
    A_x: jax.Array,
    A_k_cache: jax.Array,
    A_v_cache: jax.Array,
    A_wq: jax.Array,
    A_wo: jax.Array,
    B_x: jax.Array,
    B_k_cache: jax.Array,
    B_v_cache: jax.Array,
    B_wq: jax.Array,
    B_wo: jax.Array,
):
    anyspec = pl.BlockSpec(memory_space=pl.ANY)
    return pl.pallas_call(
        functools.partial(kern, scopes=0, endq=1),
        in_specs=[anyspec] * 10,
        out_specs=anyspec,
        out_shape=jax.ShapeDtypeStruct((B, SQ, 2 * D), BF),
        scratch_shapes=[
            pltpu.VMEM((2, B, SQ, D), BF),
            pltpu.VMEM((2, B, H, SK, DH), BF),
            pltpu.VMEM((2, B, H, SK, DH), BF),
            pltpu.VMEM((2, NG, D, W), BF),
            pltpu.VMEM((2, H * DH, D), BF),
            pltpu.VMEM((NT, M, D), F32),
            pltpu.VMEM((2, B, SQ, D), BF),
            pltpu.VMEM((2, BB, HG, SQ, DH), BF),
            pltpu.VMEM((M, W), BF),
            pltpu.SemaphoreType.DMA((NSEM,)),
        ],
        compiler_params=pltpu.CompilerParams(vmem_limit_bytes=110 * 1024 * 1024, disable_semaphore_checks=True),
    )(A_x, A_k_cache, A_v_cache, A_wq, A_wo, B_x, B_k_cache, B_v_cache, B_wq, B_wo)
```

```python
import functools
import math

import jax
import jax.numpy as jnp
from jax import lax
import jax.experimental.pallas as pl
import jax.experimental.pallas.tpu as pltpu

B, SQ, D = 32, 48, 512
H, SK, DH = 32, 48, 128
C2 = (DH ** -0.5) * math.log2(math.e)
BB = 4
HG = 4
NT = B // BB
NG = H // HG
W = HG * DH
M = BB * SQ
NTILES = 2 * NT * NG
BF = jnp.bfloat16
F32 = jnp.float32
PRO, L, EPI = 16, 12, 4
NB = (NTILES - PRO - EPI) // L
NA = 4
OSPLIT = 4

PLAN = [
    ("x0:1 qa", "a0"),
    ("x1:1", "a1"),
    ("qb", "b0 b1"),
    ("x2:3", "Q2 Q3 Q4"),
    ("q1 x5:3", "Q8 Q9 Q10 Q11 Q12 Q5 Q6 Q7 Q13 Q14"),
    ("k0 v0 o0",
     "S0 Q15 S1 P0 S2 O0 P1 S3 O1 P2 S4 O2 P3 S5 O3 P4 S6 O4 P5 S7 P6 O5"),
    ("k1 v1 o1 q2",
     "P7 S8 O6 S9 O7 P8 S10 Q16 P9 O8 S11 O9 P10 S12 O10 P11 S13 O11 P12 S14 O12 "
     "P13 S15 O13 P14 Q17 O14"),
]
EPILOGUE = "P123 S124 Q126 S125 Q127 P124 S126 O123 P125 S127 O124 P126 O125 P127 O126"
S_BLK = len(PLAN)
S_EP = S_BLK + NB
S_OUT = S_EP + 1
NSEM = S_OUT + 1


def _tile_coords(i):
    if isinstance(i, int):
        br, hi, lo = i >> 6, (i >> 3) & 7, i & 7
        return (br, lo, hi) if br == 0 else (br, hi, lo)
    br = lax.shift_right_logical(i, 6)
    hi = lax.shift_right_logical(i, 3) & 7
    lo = i & 7
    return br, jnp.where(br == 0, lo, hi), jnp.where(br == 0, hi, lo)


def _kernel(ax, ak, av, awq, awo, bx, bk, bv, bwq, bwo, out_hbm,
            x_buf, k_buf, v_buf, wq_buf, wo_buf, acc_ref, stage, q_car, p_car, sem):
    def cp(src, dst, s):
        return pltpu.make_async_copy(src, dst, sem.at[s])

    def x_a(t0, n, s):
        rows = pl.ds(t0 * BB, n * BB)
        return cp(ax.at[rows], x_buf.at[0, rows], s)

    def kv_a(which, g, half, nhalf, s):
        src, buf = ((ak, k_buf), (av, v_buf))[which]
        rows = pl.ds(half * (B // 2), nhalf * (B // 2))
        heads = pl.ds(g * HG, HG)
        return cp(src.at[rows, heads], buf.at[0, rows, heads], s)

    def kv_b(which, t, half, nhalf, s):
        src, buf = ((bk, k_buf), (bv, v_buf))[which]
        rows = pl.ds(t * BB, BB)
        heads = pl.ds(half * (H // 2), nhalf * (H // 2))
        return cp(src.at[rows, heads], buf.at[1, rows, heads], s)

    def wq_c(br, g, s, c0=0, cn=W):
        return cp((awq, bwq)[br].at[:, pl.ds(g * W + c0, cn)],
                  wq_buf.at[br, g, :, pl.ds(c0, cn)], s)

    def wo_a(g, s):
        return cp(awo.at[pl.ds(g * W, W)], wo_buf.at[0, pl.ds(g * W, W)], s)

    def blk_kv(jj, fn, u0, s):
        odd = jj & 1
        u = u0 + ((3 * jj) >> 1)
        return ([fn(w, u + odd, 0, 2, s) for w in range(2)]
                + [fn(w, u + 1 - odd, odd, 1, s) for w in range(2)])

    def blk_a(j):
        s = S_BLK + j
        wq_g, wo_g = [((3,), (2, 3)), ((4, 5), (4,)), ((6,), (5, 6)), ((7,), (7,))][j]
        return (blk_kv(j, kv_a, PRO // NT, s)
                + [wq_c(0, g, s) for g in wq_g] + [wo_a(g, s) for g in wo_g])

    def b_weights():
        s = S_BLK + NA - 1
        return ([cp(bx, x_buf.at[1], s), cp(bwo, wo_buf.at[1], s)]
                + [wq_c(1, g, s) for g in range(NG)])

    def blk_b(j):
        return blk_kv(j - NA, kv_b, 0, S_BLK + j)

    def ep_kv():
        return [kv_b(w, NT - 1, 1, 1, S_EP) for w in range(2)]

    def out_a():
        return cp(stage.at[0], out_hbm.at[:, :, pl.ds(0, D)], S_OUT)

    def group(n):
        res = []
        for tok in PLAN[n][0].split():
            c, rest = tok[0], tok[1:]
            if c == "x":
                t0, cnt = rest.split(":")
                res.append(x_a(int(t0), int(cnt), n))
            elif tok in ("qa", "qb"):
                res.append(wq_c(0, 0, n, (W // 2) * (tok == "qb"), W // 2))
            elif c == "q":
                res.append(wq_c(0, int(rest), n))
            elif c == "o":
                res.append(wo_a(int(rest), n))
            else:
                res.append(kv_a("kv".index(c), int(rest), 0, 2, n))
        return res

    def start(copies):
        for c in copies:
            c.start()

    def wait(copies):
        for c in copies:
            c.wait()

    q, pr, o = {}, {}, {}

    def stage_q(i, key, h0=0, nh=HG):
        br, t, g = _tile_coords(i)
        x = x_buf[br, pl.ds(t * BB, BB)].reshape(M, D)
        qq = jnp.dot(x, wq_buf[br, g, :, h0 * DH:(h0 + nh) * DH], preferred_element_type=F32)
        d = q.setdefault(key, {})
        for hh in range(nh):
            for b in range(BB):
                d[b, h0 + hh] = qq[b * SQ:(b + 1) * SQ, hh * DH:(hh + 1) * DH].astype(BF)

    def stage_s(i, key):
        br, t, g = _tile_coords(i)
        qs = q.pop(key)
        d = {}
        for hh in range(HG):
            for b in range(BB):
                s = lax.dot_general(qs[b, hh], k_buf[br, t * BB + b, g * HG + hh],
                                    (((1,), (1,)), ((), ())), preferred_element_type=F32)
                m = jnp.max(s, axis=-1, keepdims=True)
                e = jnp.exp2((s - m) * C2)
                l = jnp.sum(e, axis=-1, keepdims=True)
                d[b, hh] = (e * pl.reciprocal(l, approx=False, full_range=False)).astype(BF)
        pr[key] = d

    def stage_p(i, key, coords=None):
        if coords is None:
            br, t, g = _tile_coords(i)
            b0, h0 = t * BB, g * HG
        else:
            br, b0, h0 = coords
        ps = pr.pop(key)
        d = {}
        for hh in range(HG):
            for b in range(BB):
                d[b, hh] = jnp.dot(ps[b, hh], v_buf[br, b0 + b, h0 + hh],
                                   preferred_element_type=F32).astype(BF)
        rows = [jnp.concatenate([d[b, hh] for hh in range(HG)], axis=1) for b in range(BB)]
        o[key] = jnp.concatenate(rows, axis=0)

    def stage_o(i, key):
        br, t, g = _tile_coords(i)
        if isinstance(i, int):
            assert g < NG - 1
            p = jnp.dot(o.pop(key), wo_buf[br, g * W:(g + 1) * W], preferred_element_type=F32)
            acc_ref[t] = p if g == 0 else acc_ref[t] + p
        else:
            p = jnp.dot(o.pop(key), wo_buf[br, pl.ds(pl.multiple_of(g * W, W), W)],
                        preferred_element_type=F32)
            a = jnp.where(g == 0, 0.0, acc_ref[t]) + p
            acc_ref[t] = a
            stage[br, pl.ds(t * BB, BB)] = a.astype(BF).reshape(BB, SQ, D)

    def save_carry(k0):
        for j in range(2):
            for (b, hh), val in q.pop(k0 + j).items():
                q_car[j, b, hh] = val
        for (b, hh), val in pr.pop(k0 - 1).items():
            p_car[b, hh] = val

    def load_carry(k0):
        for j in range(2):
            q[k0 + j] = {(b, hh): q_car[j, b, hh] for hh in range(HG) for b in range(BB)}
        pr[k0 - 1] = {(b, hh): p_car[b, hh] for hh in range(HG) for b in range(BB)}

    def run_seq(seq):
        for tok in seq.split():
            i = int(tok[1:])
            if tok[0] in "ab":
                stage_q(i, i, (HG // 2) * (tok[0] == "b"), HG // 2)
            else:
                {"Q": stage_q, "S": stage_s, "P": stage_p, "O": stage_o}[tok[0]](i, i)

    def prologue():
        for n in range(len(PLAN)):
            wait(group(n))
            run_seq(PLAN[n][1])
            if n == len(PLAN) - 3:
                start(b_weights())
                for j in range(NA, NB):
                    start(blk_b(j))
                start(ep_kv())
        save_carry(PRO)
        wait(blk_a(0))

    def block(j, coords):
        preds = [j == ja for ja in range(1, NA)]
        pred_b = j >= NA
        for ja in range(1, NA):
            @pl.when(preds[ja - 1])
            def _():
                wait(blk_a(ja) + (b_weights() if ja == NA - 1 else []))

        @pl.when(pred_b)
        def _():
            wait(blk_b(j))

        base = PRO + j * L
        load_carry(0)
        for k in range(L):
            i = base + k
            stage_p(i - 1, k - 1, coords if k == 0 else None)
            stage_s(i, k)
            stage_o(i - 1, k - 1)
            stage_q(i + 2, k + 2)
        save_carry(L)

        @pl.when(j == NA)
        def _():
            out_a().start()

    def epilogue():
        wait(ep_kv())
        nb7 = (NT - 1) * BB
        outs = [cp(stage.at[1, pl.ds(0, nb7)],
                   out_hbm.at[pl.ds(0, nb7), :, pl.ds(D, D)], S_OUT)]
        outs[0].start()
        load_carry(NTILES - EPI)
        run_seq(EPILOGUE)
        cw = D // OSPLIT
        o_last = o.pop(NTILES - 1)
        for c in range(OSPLIT):
            cols = slice(c * cw, (c + 1) * cw)
            p = jnp.dot(o_last, wo_buf[1, (NG - 1) * W:NG * W, cols], preferred_element_type=F32)
            stage[1, nb7:B, :, cols] = (acc_ref[NT - 1, :, cols] + p).astype(BF).reshape(BB, SQ, cw)
            piece = cp(stage.at[1, pl.ds(nb7, BB), :, pl.ds(c * cw, cw)],
                       out_hbm.at[pl.ds(nb7, BB), :, pl.ds(D + c * cw, cw)], S_OUT)
            piece.start()
            outs.append(piece)
        wait([out_a()] + outs)

    for n in range(len(PLAN)):
        start(group(n))
    for j in range(NA):
        start(blk_a(j))

    def body(j, coords):
        pl.when(j == 0)(prologue)
        block(j, coords)
        pl.when(j == NB - 1)(epilogue)
        br, t, g = _tile_coords(PRO + j * L + L - 1)
        return br, t * BB, g * HG

    br0, t0, g0 = _tile_coords(PRO - 1)
    lax.fori_loop(0, NB, body, (jnp.int32(br0), jnp.int32(t0 * BB), jnp.int32(g0 * HG)))


def _call(args, interpret=False):
    anyspec = pl.BlockSpec(memory_space=pl.ANY)
    return pl.pallas_call(
        _kernel,
        in_specs=[anyspec] * 10,
        out_specs=anyspec,
        out_shape=jax.ShapeDtypeStruct((B, SQ, 2 * D), BF),
        scratch_shapes=[
            pltpu.VMEM((2, B, SQ, D), BF),
            pltpu.VMEM((2, B, H, SK, DH), BF),
            pltpu.VMEM((2, B, H, SK, DH), BF),
            pltpu.VMEM((2, NG, D, W), BF),
            pltpu.VMEM((2, H * DH, D), BF),
            pltpu.VMEM((NT, M, D), F32),
            pltpu.VMEM((2, B, SQ, D), BF),
            pltpu.VMEM((2, BB, HG, SQ, DH), BF),
            pltpu.VMEM((BB, HG, SQ, SK), BF),
            pltpu.SemaphoreType.DMA((NSEM,)),
        ],
        compiler_params=pltpu.CompilerParams(
            vmem_limit_bytes=110 * 1024 * 1024,
            disable_semaphore_checks=True,
        ),
        interpret=interpret,
    )(*args)


@jax.jit
def pallas_concat_heads__gqa_block_cached__gqa_block_cached__near_ridge_kernel(
    A_x: jax.Array,
    A_k_cache: jax.Array,
    A_v_cache: jax.Array,
    A_wq: jax.Array,
    A_wo: jax.Array,
    B_x: jax.Array,
    B_k_cache: jax.Array,
    B_v_cache: jax.Array,
    B_wq: jax.Array,
    B_wo: jax.Array,
):
    return _call((A_x, A_k_cache, A_v_cache, A_wq, A_wo,
                  B_x, B_k_cache, B_v_cache, B_wq, B_wo))
```

```python
import jax
import jax.numpy as jnp
from jax import lax
import jax.experimental.pallas as pl
import jax.experimental.pallas.tpu as pltpu

B, SQ, D = 32, 48, 512
H, SK, DH = 32, 48, 128
BB = 4
HG = 4
NT = B // BB
NG = H // HG
W = HG * DH
M = BB * SQ
NTILES = 2 * NT * NG
BF = jnp.bfloat16
F32 = jnp.float32
PRO, L, EPI = 16, 12, 4
NB = (NTILES - PRO - EPI) // L
NA = 4
OSPLIT = 4

PLAN = [
    ("x0:1 qa", "a0"),
    ("x1:1", "a1"),
    ("qb", "b0 b1"),
    ("x2:3", "Q2 Q3 Q4"),
    ("q1 x5:3", "Q8 Q9 Q10 Q11 Q12 Q5 Q6 Q7 Q13 Q14"),
    ("k0 v0 o0",
     "S0 Q15 S1 P0 S2 O0 P1 S3 O1 P2 S4 O2 P3 S5 O3 P4 S6 O4 P5 S7 P6 O5"),
    ("k1 v1 o1 q2",
     "P7 S8 O6 S9 O7 P8 S10 Q16 P9 O8 S11 O9 P10 S12 O10 P11 S13 O11 P12 S14 O12 "
     "P13 S15 O13 P14 Q17 O14"),
]
EPILOGUE = "P123 S124 Q126 S125 Q127 P124 S126 O123 P125 S127 O124 P126 O125 P127 O126"
S_BLK = len(PLAN)
S_EP = S_BLK + NB
S_OUT = S_EP + 1
NSEM = S_OUT + 1


def _tile_coords(i):
    if isinstance(i, int):
        br, hi, lo = i >> 6, (i >> 3) & 7, i & 7
        return (br, lo, hi) if br == 0 else (br, hi, lo)
    br = lax.shift_right_logical(i, 6)
    hi = lax.shift_right_logical(i, 3) & 7
    lo = i & 7
    return br, jnp.where(br == 0, lo, hi), jnp.where(br == 0, hi, lo)


def _kernel(ax, ak, av, awq, awo, bx, bk, bv, bwq, bwo, out_hbm,
            x_buf, k_buf, v_buf, wq_buf, wo_buf, acc_ref, stage, q_car, p_car, sem):
    def cp(src, dst, s):
        return pltpu.make_async_copy(src, dst, sem.at[s])

    def x_a(t0, n, s):
        rows = pl.ds(t0 * BB, n * BB)
        return cp(ax.at[rows], x_buf.at[0, rows], s)

    def kv_a_rows(which, g, b0, nb, s):
        src, buf = ((ak, k_buf), (av, v_buf))[which]
        rows, heads = pl.ds(b0, nb), pl.ds(g * HG, HG)
        return cp(src.at[rows, heads], buf.at[0, rows, heads], s)

    def kv_a(which, g, half, nhalf, s):
        cut = B // 2
        if which == 1 and g == 3:
            cut -= BB
        b0 = cut * half
        b1 = B if half + nhalf == 2 else cut
        return kv_a_rows(which, g, b0, b1 - b0, s)

    def kv_b(which, t, half, nhalf, s):
        src, buf = ((bk, k_buf), (bv, v_buf))[which]
        rows = pl.ds(t * BB, BB)
        heads = pl.ds(half * (H // 2), nhalf * (H // 2))
        return cp(src.at[rows, heads], buf.at[1, rows, heads], s)

    def wq_c(br, g, s, c0=0, cn=W):
        return cp((awq, bwq)[br].at[:, pl.ds(g * W + c0, cn)],
                  wq_buf.at[br, g, :, pl.ds(c0, cn)], s)

    def wo_a(g, s):
        return cp(awo.at[pl.ds(g * W, W)], wo_buf.at[0, pl.ds(g * W, W)], s)

    def blk_kv(jj, fn, u0, s):
        odd = jj & 1
        u = u0 + ((3 * jj) >> 1)
        return ([fn(w, u + odd, 0, 2, s) for w in range(2)]
                + [fn(w, u + 1 - odd, odd, 1, s) for w in range(2)])

    def blk_a(j):
        s = S_BLK + j
        wq_g, wo_g = [((3,), (2, 3)), ((4, 5), (4,)), ((6,), (5, 6)), ((7,), (7,))][j]
        return (blk_kv(j, kv_a, PRO // NT, s)
                + [wq_c(0, g, s) for g in wq_g] + [wo_a(g, s) for g in wo_g])

    def b_weights():
        s = S_BLK + NA - 1
        return ([cp(bx, x_buf.at[1], s), cp(bwo, wo_buf.at[1], s)]
                + [wq_c(1, g, s) for g in range(NG)])

    def blk_b(j):
        return blk_kv(j - NA, kv_b, 0, S_BLK + j)

    def ep_kv():
        return [kv_b(w, NT - 1, 1, 1, S_EP) for w in range(2)]

    def out_a():
        return cp(stage.at[0], out_hbm.at[:, :, pl.ds(0, D)], S_OUT)

    def group(n):
        res = []
        for tok in PLAN[n][0].split():
            c, rest = tok[0], tok[1:]
            if c == "x":
                t0, cnt = rest.split(":")
                res.append(x_a(int(t0), int(cnt), n))
            elif tok in ("qa", "qb"):
                res.append(wq_c(0, 0, n, (W // 2) * (tok == "qb"), W // 2))
            elif c == "q":
                res.append(wq_c(0, int(rest), n))
            elif c == "o":
                res.append(wo_a(int(rest), n))
            else:
                res.append(kv_a("kv".index(c), int(rest), 0, 2, n))
        return res

    def start(copies):
        for c in copies:
            c.start()

    def wait(copies):
        for c in copies:
            c.wait()

    q, pr, o = {}, {}, {}

    def stage_q(i, key, h0=0, nh=HG):
        br, t, g = _tile_coords(i)
        x = x_buf[br, pl.ds(t * BB, BB)].reshape(M, D)
        qq = jnp.dot(x, wq_buf[br, g, :, h0 * DH:(h0 + nh) * DH], preferred_element_type=F32)
        d = q.setdefault(key, {})
        for hh in range(nh):
            for b in range(BB):
                d[b, h0 + hh] = qq[b * SQ:(b + 1) * SQ, hh * DH:(hh + 1) * DH].astype(BF)

    def stage_s(i, key):
        br, t, g = _tile_coords(i)
        qs = q.pop(key)
        d = {}
        for hh in range(HG):
            for b in range(BB):
                s = lax.dot_general(qs[b, hh], k_buf[br, t * BB + b, g * HG + hh],
                                    (((1,), (1,)), ((), ())), preferred_element_type=F32)
                s = (s.astype(BF) * (DH ** -0.5)).astype(F32)
                m = jnp.max(s, axis=-1, keepdims=True)
                e = jnp.exp(s - m)
                l = jnp.sum(e, axis=-1, keepdims=True)
                d[b, hh] = (e * pl.reciprocal(l, approx=False, full_range=False)).astype(BF)
        pr[key] = d

    def stage_p(i, key, coords=None):
        if coords is None:
            br, t, g = _tile_coords(i)
            b0, h0 = t * BB, g * HG
        else:
            br, b0, h0 = coords
        ps = pr.pop(key)
        d = {}
        for hh in range(HG):
            for b in range(BB):
                d[b, hh] = jnp.dot(ps[b, hh], v_buf[br, b0 + b, h0 + hh],
                                   preferred_element_type=F32).astype(BF)
        rows = [jnp.concatenate([d[b, hh] for hh in range(HG)], axis=1) for b in range(BB)]
        o[key] = jnp.concatenate(rows, axis=0)

    def stage_o(i, key):
        br, t, g = _tile_coords(i)
        if isinstance(i, int):
            assert g < NG - 1
            p = jnp.dot(o.pop(key), wo_buf[br, g * W:(g + 1) * W], preferred_element_type=F32)
            acc_ref[t] = p if g == 0 else acc_ref[t] + p
        else:
            p = jnp.dot(o.pop(key), wo_buf[br, pl.ds(pl.multiple_of(g * W, W), W)],
                        preferred_element_type=F32)
            a = jnp.where(g == 0, 0.0, acc_ref[t]) + p
            acc_ref[t] = a
            stage[br, pl.ds(t * BB, BB)] = a.astype(BF).reshape(BB, SQ, D)

    def save_carry(k0):
        for j in range(2):
            for (b, hh), val in q.pop(k0 + j).items():
                q_car[j, b, hh] = val
        for (b, hh), val in pr.pop(k0 - 1).items():
            p_car[b, hh] = val

    def load_carry(k0):
        for j in range(2):
            q[k0 + j] = {(b, hh): q_car[j, b, hh] for hh in range(HG) for b in range(BB)}
        pr[k0 - 1] = {(b, hh): p_car[b, hh] for hh in range(HG) for b in range(BB)}

    def run_seq(seq):
        for tok in seq.split():
            i = int(tok[1:])
            if tok[0] in "ab":
                stage_q(i, i, (HG // 2) * (tok[0] == "b"), HG // 2)
            else:
                {"Q": stage_q, "S": stage_s, "P": stage_p, "O": stage_o}[tok[0]](i, i)

    def prologue():
        for n in range(len(PLAN)):
            wait(group(n))
            run_seq(PLAN[n][1])
            if n == len(PLAN) - 3:
                start(b_weights())
                for j in range(NA, NB):
                    start(blk_b(j))
                start(ep_kv())
        save_carry(PRO)
        wait(blk_a(0))

    def block(j, coords):
        preds = [j == ja for ja in range(1, NA)]
        pred_b = j >= NA
        for ja in range(1, NA):
            @pl.when(preds[ja - 1])
            def _():
                wait(blk_a(ja) + (b_weights() if ja == NA - 1 else []))

        @pl.when(pred_b)
        def _():
            wait(blk_b(j))

        base = PRO + j * L
        load_carry(0)
        for k in range(L):
            i = base + k
            stage_p(i - 1, k - 1, coords if k == 0 else None)
            stage_s(i, k)
            stage_o(i - 1, k - 1)
            stage_q(i + 2, k + 2)
        save_carry(L)

        @pl.when(j == NA)
        def _():
            out_a().start()

    def epilogue():
        wait(ep_kv())
        nb7 = (NT - 1) * BB
        outs = [cp(stage.at[1, pl.ds(0, nb7)],
                   out_hbm.at[pl.ds(0, nb7), :, pl.ds(D, D)], S_OUT)]
        outs[0].start()
        load_carry(NTILES - EPI)
        run_seq(EPILOGUE)
        cw = D // OSPLIT
        o_last = o.pop(NTILES - 1)
        for c in range(OSPLIT):
            cols = slice(c * cw, (c + 1) * cw)
            p = jnp.dot(o_last, wo_buf[1, (NG - 1) * W:NG * W, cols], preferred_element_type=F32)
            res = (acc_ref[NT - 1, :, cols] + p).astype(BF).reshape(BB, SQ, cw)
            parts = [(0, BB)] if c < OSPLIT - 1 else [(0, BB - 1), (BB - 1, 1)]
            for b0, nb in parts:
                stage[1, nb7 + b0:nb7 + b0 + nb, :, cols] = res[b0:b0 + nb]
                piece = cp(stage.at[1, pl.ds(nb7 + b0, nb), :, pl.ds(c * cw, cw)],
                           out_hbm.at[pl.ds(nb7 + b0, nb), :, pl.ds(D + c * cw, cw)], S_OUT)
                piece.start()
                outs.append(piece)
        wait([out_a()] + outs)

    for n in range(len(PLAN)):
        start(group(n))
    for j in range(NA):
        start(blk_a(j))

    def body(j, coords):
        block(j, coords)
        br, t, g = _tile_coords(PRO + j * L + L - 1)
        return br, t * BB, g * HG

    def everything():
        prologue()
        br0, t0, g0 = _tile_coords(PRO - 1)
        lax.fori_loop(0, NB, body, (jnp.int32(br0), jnp.int32(t0 * BB), jnp.int32(g0 * HG)))
        epilogue()

    def outer(it, c):
        pl.when(it == 1)(everything)
        return c

    lax.fori_loop(0, 2, outer, 0)


@jax.jit
def pallas_concat_heads__gqa_block_cached__gqa_block_cached__near_ridge_kernel(
    A_x: jax.Array,
    A_k_cache: jax.Array,
    A_v_cache: jax.Array,
    A_wq: jax.Array,
    A_wo: jax.Array,
    B_x: jax.Array,
    B_k_cache: jax.Array,
    B_v_cache: jax.Array,
    B_wq: jax.Array,
    B_wo: jax.Array,
):
    anyspec = pl.BlockSpec(memory_space=pl.ANY)
    return pl.pallas_call(
        _kernel,
        in_specs=[anyspec] * 10,
        out_specs=anyspec,
        out_shape=jax.ShapeDtypeStruct((B, SQ, 2 * D), BF),
        scratch_shapes=[
            pltpu.VMEM((2, B, SQ, D), BF),
            pltpu.VMEM((2, B, H, SK, DH), BF),
            pltpu.VMEM((2, B, H, SK, DH), BF),
            pltpu.VMEM((2, NG, D, W), BF),
            pltpu.VMEM((2, H * DH, D), BF),
            pltpu.VMEM((NT, M, D), F32),
            pltpu.VMEM((2, B, SQ, D), BF),
            pltpu.VMEM((2, BB, HG, SQ, DH), BF),
            pltpu.VMEM((BB, HG, SQ, SK), BF),
            pltpu.SemaphoreType.DMA((NSEM,)),
        ],
        compiler_params=pltpu.CompilerParams(
            vmem_limit_bytes=110 * 1024 * 1024,
            disable_semaphore_checks=True,
        ),
    )(A_x, A_k_cache, A_v_cache, A_wq, A_wo,
      B_x, B_k_cache, B_v_cache, B_wq, B_wo)
```
